```python
import os as _os
_os.environ.setdefault("JAX_PLATFORMS", "cpu")
import jax
import jax.numpy as jnp

def _softmax(x, axis=-1):
    return jax.nn.softmax(x, axis=axis)
def _gelu(x):
    return jax.nn.gelu(x, approximate=True)
def _silu(x):
    return jax.nn.silu(x)
def _sigmoid(x):
    return jax.nn.sigmoid(x)
def _layernorm(x, axis=-1, eps=1e-5):
    m = jnp.mean(x, axis=axis, keepdims=True)
    v = jnp.var(x, axis=axis, keepdims=True)
    return (x - m) / jnp.sqrt(v + eps)
def _scatter_add(tgt, idx, src, axis=0):
    return tgt.at[idx].add(src)
def _segment_sum(src, seg, n):
    return jax.ops.segment_sum(src, seg, n)
class _Rng:
    def __init__(self, key):
        self._k = key
    def _next(self):
        self._k, sub = jax.random.split(self._k)
        return sub
    def normal(self, shape):
        return jax.random.normal(self._next(), shape, dtype=jnp.bfloat16)
    def randint(self, lo, hi, shape):
        return jax.random.randint(self._next(), shape, lo, hi, dtype=jnp.int32)
    def uniform(self, shape, lo=0.0, hi=1.0):
        return jax.random.uniform(self._next(), shape, jnp.bfloat16, lo, hi)
    def permutation(self, n):
        return jax.random.permutation(self._next(), n)


kernel_name = 'standalone__sliding_block_cached__sampling'

def setup_inputs():
    _rng = _Rng(jax.random.key(int.from_bytes(__import__("os").urandom(4), "little")))
    _w = (lambda a: (lambda t: t.astype(jnp.bfloat16) if jnp.issubdtype(t.dtype, jnp.floating) else t)(jnp.asarray(a)))
    B, Sq, D = 8, 4, 640
    Hq, Hkv, Sk, Dh = 32, 32, 4096, 192
    assert Hq % Hkv == 0, (Hq, Hkv)
    return {
        "x": _w((lambda *s: _rng.normal(s) * 0.8)(B, Sq, D)),
        "k_cache": _w((lambda *s: _rng.normal(s) * 0.8)(B, Hkv, Sk, Dh)),
        "v_cache": _w((lambda *s: _rng.normal(s) * 0.05)(B, Hkv, Sk, Dh)),
        "wq": _w((lambda *s: _rng.normal(s) * 0.8)(D, Hq * Dh) * (D ** -0.5)),
        "wo": _w((lambda *s: _rng.normal(s) * 0.05)(Hq * Dh, D) * ((Hq * Dh) ** -0.5)),
    }

def reference(x, k_cache, v_cache, wq, wo):
    B, Sq, D = x.shape
    Hq, Dh = 32, 192
    Hkv, Sk = k_cache.shape[1], k_cache.shape[2]
    W = min(4096, max(256, Sk // 4))
    rep = Hq // Hkv
    q = (lambda x, *d: x.transpose(*d))((x @ wq).reshape(B, Sq, Hq, Dh), 0, 2, 1, 3)
    k = jnp.repeat(k_cache[:, :, Sk - W:, :], rep, axis=1)
    v = jnp.repeat(v_cache[:, :, Sk - W:, :], rep, axis=1)
    scores = jnp.einsum("bhqd,bhkd->bhqk", q, k) * (Dh ** -0.5)
    p = _softmax(scores, axis=-1)
    o = jnp.einsum("bhqk,bhkd->bhqd", p, v)
    return (lambda x, *d: x.transpose(*d))(o, 0, 2, 1, 3).reshape(B, Sq, Hq * Dh) @ wo
```

```python
import jax
import jax.numpy as jnp
from jax import lax
import jax.experimental.pallas as pl
import jax.experimental.pallas.tpu as pltpu

_HQ, _DH = 32, 192
_DEPTH = 3
_ROWS = 8


@jax.jit
def pallas_standalone__sliding_block_cached__sampling_kernel(
    x: jax.Array,
    k_cache: jax.Array,
    v_cache: jax.Array,
    wq: jax.Array,
    wo: jax.Array,
):
    B, Sq, D = x.shape
    _, H, Sk, Dh = k_cache.shape
    assert (H, Dh) == (_HQ, _DH) and Sq == 4 and B % 2 == 0
    W = min(4096, max(256, Sk // 4))
    scale = Dh ** -0.5
    NBP = B // 2
    HP = H // 2
    n_it = H * NBP
    depth, rows = _DEPTH, _ROWS
    items = [(a, bi, r2 * 2 + g, g) for r2 in range(Dh // rows // 2) for bi in range(2)
             for a in range(2) for g in range(2)]

    def kernel_function(x_hbm, k_hbm, v_hbm, wq_hbm, wo_hbm, o_ref,
                        x_v, wq_v, wo_v, kbuf, vbuf, q_s, o_s, acc,
                        kv_sem, wq_sem, wo_sem, x_sem):
        def start_kv(i, slot):
            h, bp = i // NBP, i % NBP
            for (a, bi, r, p) in items:
                src, buf = ((k_hbm, kbuf), (v_hbm, vbuf))[a]
                pltpu.make_async_copy(
                    src.at[2 * bp + bi, h, pl.ds(r * rows, rows), pl.ds(Sk - W, W)],
                    buf.at[slot, bi, pl.ds(r * rows, rows), :],
                    kv_sem.at[a, slot]).start(priority=p)

        def wait_kv(a, slot):
            buf = (kbuf, vbuf)[a]
            pltpu.make_async_copy(buf.at[slot], buf.at[slot], kv_sem.at[a, slot]).wait()

        def wq_copy(hp):
            c0 = pl.multiple_of(hp * 2 * Dh, 128)
            return pltpu.make_async_copy(wq_hbm.at[:, pl.ds(c0, 2 * Dh)], wq_v.at[hp % 2], wq_sem.at[hp % 2])

        def wo_copy(hp):
            r0 = pl.multiple_of(hp * 2 * Dh, 128)
            return pltpu.make_async_copy(wo_hbm.at[pl.ds(r0, 2 * Dh), :], wo_v.at[hp % 2], wo_sem.at[hp % 2])

        x_copy = pltpu.make_async_copy(x_hbm, x_v, x_sem)
        x_copy.start()
        wq_copy(0).start()
        for i in range(depth):
            start_kv(i, i)
        wo_copy(0).start(priority=1)
        x_copy.wait()
        xf = x_v[...].astype(jnp.float32).reshape(B * Sq, D).astype(jnp.bfloat16)
        acc[...] = jnp.zeros_like(acc)
        first = lax.broadcasted_iota(jnp.int32, (8, 1), 0) < Sq

        def head_pair(hp, carry):
            @pl.when(hp + 1 < HP)
            def _():
                wq_copy(hp + 1).start()
                wo_copy(hp + 1).start(priority=1)
            wq_copy(hp).wait()
            q = jnp.dot(xf, wq_v[hp % 2], preferred_element_type=jnp.float32)
            q = q.astype(jnp.bfloat16).astype(jnp.float32)
            q_s[0] = q[:, :Dh]
            q_s[1] = q[:, Dh:]

            def body(j, c):
                i = hp * 2 * NBP + j
                hh, bp = j // NBP, j % NBP
                slot = i % depth
                r0 = pl.multiple_of(bp * 8, 8)
                qb = q_s[hh, pl.ds(r0, 8), :].astype(jnp.bfloat16)
                wait_kv(0, slot)
                s0 = jnp.dot(qb, kbuf[slot, 0], preferred_element_type=jnp.float32)
                s1 = jnp.dot(qb, kbuf[slot, 1], preferred_element_type=jnp.float32)
                s = jnp.where(first, s0, s1) * scale
                m = jnp.max(s, axis=1, keepdims=True)
                e = jnp.exp(s - m)
                l = jnp.sum(e, axis=1, keepdims=True)
                p = e.astype(jnp.bfloat16)
                wait_kv(1, slot)
                dn = (((1,), (1,)), ((), ()))
                o0 = lax.dot_general(p, vbuf[slot, 0], dn, preferred_element_type=jnp.float32)
                o1 = lax.dot_general(p, vbuf[slot, 1], dn, preferred_element_type=jnp.float32)
                o_s[hh, pl.ds(r0, 8), :] = jnp.where(first, o0, o1) / l

                @pl.when(i + depth < n_it)
                def _():
                    start_kv(i + depth, slot)
                return c

            lax.fori_loop(0, 2 * NBP, body, 0)
            wo_copy(hp).wait()
            a = acc[...]
            for hh in range(2):
                a += jnp.dot(o_s[hh].astype(jnp.bfloat16), wo_v[hp % 2, pl.ds(hh * Dh, Dh), :],
                             preferred_element_type=jnp.float32)
            acc[...] = a
            return carry

        lax.fori_loop(0, HP, head_pair, 0)
        o_ref[...] = acc[...].reshape(B, Sq, D).astype(o_ref.dtype)

    kt = jnp.swapaxes(k_cache, 2, 3)
    vt = jnp.swapaxes(v_cache, 2, 3)
    any_spec = pl.BlockSpec(memory_space=pl.ANY)
    return pl.pallas_call(
        kernel_function,
        in_specs=[any_spec] * 5,
        out_specs=pl.BlockSpec(memory_space=pltpu.VMEM),
        out_shape=jax.ShapeDtypeStruct(x.shape, x.dtype),
        scratch_shapes=[
            pltpu.VMEM((B, Sq, D), jnp.bfloat16),
            pltpu.VMEM((2, D, 2 * Dh), jnp.bfloat16),
            pltpu.VMEM((2, 2 * Dh, D), jnp.bfloat16),
            pltpu.VMEM((depth, 2, Dh, W), jnp.bfloat16),
            pltpu.VMEM((depth, 2, Dh, W), jnp.bfloat16),
            pltpu.VMEM((2, B * Sq, Dh), jnp.float32),
            pltpu.VMEM((2, B * Sq, Dh), jnp.float32),
            pltpu.VMEM((B * Sq, D), jnp.float32),
            pltpu.SemaphoreType.DMA((2, depth)),
            pltpu.SemaphoreType.DMA((2,)),
            pltpu.SemaphoreType.DMA((2,)),
            pltpu.SemaphoreType.DMA(()),
        ],
        compiler_params=pltpu.CompilerParams(vmem_limit_bytes=64 * 1024 * 1024),
    )(x, kt, vt, wq, wo)
```

```python
import jax
import jax.numpy as jnp
from jax import lax
import jax.experimental.pallas as pl
import jax.experimental.pallas.tpu as pltpu

_HQ, _DH = 32, 192
_BLK = 128
_DEPTH = 2
_WQ_STREAMS = 4
_WO_STREAMS = 3
_WO_GROUP = 2
_WO_PIECE = 32


@jax.jit
def pallas_standalone__sliding_block_cached__sampling_kernel(
    x: jax.Array,
    k_cache: jax.Array,
    v_cache: jax.Array,
    wq: jax.Array,
    wo: jax.Array,
):
    B, Sq, D = x.shape
    _, H, Sk, Dh = k_cache.shape
    W = min(4096, max(256, Sk // 4))
    scale = Dh ** -0.5
    HD = H * Dh
    PAIR = 2 * Dh
    PAIR_BLKS = PAIR // _BLK
    SLOT_BLKS = 2 * PAIR_BLKS
    n_steps = (HD // (2 * PAIR)) * B
    n_sems = 2 * _DEPTH
    stream_blks = HD // _BLK // _WO_STREAMS
    n_groups = stream_blks // _WO_GROUP
    group_rows = _WO_GROUP * _BLK
    assert (H, Dh) == (_HQ, _DH) and 2 * Sq == 8 and B % 2 == 0
    assert W % 128 == 0 and (Sk - W) % 128 == 0 and D % (16 * _WQ_STREAMS) == 0
    assert n_steps % _DEPTH == 0 and n_groups > n_sems

    def kernel_function(x_hbm, k_hbm, v_hbm, wq_hbm, wo_hbm, o_ref,
                        x_v, wq_v, wo_v, k_buf, v_buf, q_s, o_s, ring_sem, aux_sem):

        def wait_filled(view, sem):
            pltpu.make_async_copy(view, view, sem).wait()

        def start_wq():
            def rows(r, carry):
                r0 = pl.multiple_of(r * 8, 8)
                for c in range(0, HD, 2048):
                    for s in range(0, _WQ_STREAMS, 2):
                        for g in range(2):
                            at = (pl.ds(s, 2), pl.ds(r0, 8), pl.ds(c + g * 1024, 1024))
                            pltpu.make_async_copy(
                                wq_hbm.at[at], wq_v.at[at], aux_sem.at[0]).start(priority=g)
                return carry
            lax.fori_loop(0, D // _WQ_STREAMS // 8, rows, 0)

        def start_window(which, step, slot):
            src, buf = ((k_hbm, k_buf), (v_hbm, v_buf))[which]
            b, blk = step % B, (step // B) * SLOT_BLKS
            for r in range(0, _BLK, 16):
                for j in range(0, SLOT_BLKS, 2):
                    for g in range(2):
                        rows = pl.ds(r + 8 * g, 8)
                        pltpu.make_async_copy(
                            src.at[b, pl.ds(blk + j, 2), rows, pl.ds(Sk - W, W)],
                            buf.at[slot, pl.ds(j, 2), rows, :],
                            ring_sem.at[2 * slot + which]).start(priority=g)

        def start_wo(r0, n_rows, sem):
            for r in range(0, n_rows, 2 * _WO_PIECE):
                for s in range(_WO_STREAMS):
                    for g in range(2):
                        first = r0 + r + g * _WO_PIECE
                        if not isinstance(first, int):
                            first = pl.multiple_of(first, _WO_PIECE)
                        at = (s, pl.ds(first, _WO_PIECE), slice(None))
                        pltpu.make_async_copy(
                            wo_hbm.at[at], wo_v.at[at], sem).start(priority=g)

        def refill(which, step, slot):
            @pl.when(step + _DEPTH < n_steps)
            def _():
                start_window(which, step + _DEPTH, slot)

            @pl.when(step + _DEPTH >= n_steps)
            def _():
                group = 2 * slot + which
                start_wo(group * group_rows, group_rows, ring_sem.at[group])

        def iota(shape, dim):
            return lax.broadcasted_iota(jnp.int32, shape, dim)

        x_copy = pltpu.make_async_copy(x_hbm, x_v, aux_sem.at[1])
        x_copy.start()
        start_wq()

        def first_windows(slot, carry):
            start_window(0, slot, slot)
            start_window(1, slot, slot)
            return carry
        lax.fori_loop(0, _DEPTH, first_windows, 0)

        x_copy.wait()
        wait_filled(wq_v, aux_sem.at[0])
        xf = x_v[...].astype(jnp.float32)
        x2 = jnp.concatenate([xf, xf], axis=1).reshape(2 * B * Sq, D).astype(x_v.dtype)

        def attend(step, carry):
            slot = step % _DEPTH
            b, quad = step % B, step // B

            @pl.when(b == 0)
            def _():
                c0 = pl.multiple_of(quad * 2 * PAIR, 128)
                w = wq_v[:, :, pl.ds(c0, 2 * PAIR)].reshape(D, 2 * PAIR)
                q = jnp.dot(x2, w, preferred_element_type=jnp.float32)
                own = (iota(q.shape, 0) % (2 * Sq) < Sq) == (iota(q.shape, 1) % PAIR < Dh)
                q_s[...] = jnp.where(own, q, 0.0)

            q_rows = pl.ds(pl.multiple_of(b * 2 * Sq, 8), 2 * Sq)
            wait_filled(k_buf.at[slot], ring_sem.at[2 * slot])
            probs, sums = [], []
            for p in range(2):
                q = q_s[q_rows, pl.ds(p * PAIR, PAIR)].astype(k_buf.dtype)
                kt = k_buf[slot, pl.ds(p * PAIR_BLKS, PAIR_BLKS)].reshape(PAIR, W)
                s = jnp.dot(q, kt, preferred_element_type=jnp.float32) * scale
                e = jnp.exp(s - jnp.max(s, axis=1, keepdims=True))
                sums.append(jnp.sum(e, axis=1, keepdims=True))
                probs.append(e.astype(v_buf.dtype))
            refill(0, step, slot)

            odd = b % 2
            in_place = jnp.where(iota((2 * Sq, PAIR), 1) < Dh, 0, 1) == odd
            mine = jnp.where(iota((2 * Sq, _BLK), 0) < Sq, 0, 1) == odd
            o_rows = pl.ds(pl.multiple_of((b // 2) * 2 * Sq, 8), 2 * Sq)
            wait_filled(v_buf.at[slot], ring_sem.at[2 * slot + 1])
            for p in range(2):
                vt = v_buf[slot, pl.ds(p * PAIR_BLKS, PAIR_BLKS)].reshape(PAIR, W)
                o = lax.dot_general(probs[p], vt, (((1,), (1,)), ((), ())),
                                    preferred_element_type=jnp.float32) / sums[p]
                o = jnp.where(in_place, o, pltpu.roll(o, Sq, 0))
                for u in range(PAIR_BLKS):
                    pltpu.store(o_s.at[quad * SLOT_BLKS + p * PAIR_BLKS + u, o_rows, :],
                                o[:, u * _BLK:(u + 1) * _BLK], mask=mine)
            refill(1, step, slot)
            return carry
        lax.fori_loop(0, n_steps, attend, 0)

        last = (n_groups - 1) * _WO_GROUP
        last_sems = (ring_sem.at[(n_groups - 1) % n_sems], aux_sem.at[0])

        def project(acc, blk, n_blks, sem, once_arrived=None):
            def row(u):
                r = (blk + u) * _BLK
                return r if isinstance(r, int) else pl.multiple_of(r, _BLK)
            tiles = [(s, u) for s in range(_WO_STREAMS) for u in range(n_blks)]
            lhs = [o_s[s * stream_blks + blk + u].astype(wo_v.dtype) for s, u in tiles]
            wait_filled(wo_v.at[:, pl.ds(row(0), n_blks * _BLK), :], sem)
            if once_arrived is not None:
                once_arrived()
            for (s, u), o in zip(tiles, lhs):
                acc += jnp.dot(o, wo_v[s, pl.ds(row(u), _BLK), :],
                               preferred_element_type=jnp.float32)
            return acc

        def project_group(group, acc):
            sem = ring_sem.at[group % n_sems]

            def fetch_next():
                @pl.when(group + n_sems < n_groups - 1)
                def _():
                    start_wo((group + n_sems) * group_rows, group_rows, sem)

                @pl.when(group + n_sems == n_groups - 1)
                def _():
                    for u in range(_WO_GROUP):
                        start_wo((last + u) * _BLK, _BLK, last_sems[u])
            return project(acc, group * _WO_GROUP, _WO_GROUP, sem, fetch_next)

        acc = lax.fori_loop(0, n_groups - 1, project_group,
                            jnp.zeros((B * Sq, D), jnp.float32))
        for u in range(_WO_GROUP):
            acc = project(acc, last + u, 1, last_sems[u])
        o_ref[...] = acc.reshape(B, Sq, D).astype(o_ref.dtype)

    def as_blocks(cache):
        return jnp.swapaxes(cache, 2, 3).reshape(B, HD // _BLK, _BLK, Sk)

    return pl.pallas_call(
        kernel_function,
        in_specs=[pl.BlockSpec(memory_space=pl.ANY)] * 5,
        out_specs=pl.BlockSpec(memory_space=pltpu.VMEM),
        out_shape=jax.ShapeDtypeStruct(x.shape, x.dtype),
        scratch_shapes=[
            pltpu.VMEM((B, Sq, D), x.dtype),
            pltpu.VMEM((_WQ_STREAMS, D // _WQ_STREAMS, HD), wq.dtype),
            pltpu.VMEM((_WO_STREAMS, HD // _WO_STREAMS, D), wo.dtype),
            pltpu.VMEM((_DEPTH, SLOT_BLKS, _BLK, W), k_cache.dtype),
            pltpu.VMEM((_DEPTH, SLOT_BLKS, _BLK, W), v_cache.dtype),
            pltpu.VMEM((2 * B * Sq, 2 * PAIR), jnp.float32),
            pltpu.VMEM((HD // _BLK, B * Sq, _BLK), jnp.float32),
            pltpu.SemaphoreType.DMA((n_sems,)),
            pltpu.SemaphoreType.DMA((2,)),
        ],
        compiler_params=pltpu.CompilerParams(vmem_limit_bytes=64 * 1024 * 1024),
    )(
        x,
        as_blocks(k_cache),
        as_blocks(v_cache),
        wq.reshape(_WQ_STREAMS, D // _WQ_STREAMS, HD),
        wo.reshape(_WO_STREAMS, HD // _WO_STREAMS, D),
    )
```
